```python
import jax
import jax.numpy as jnp

def _softmax(x, axis=-1):
    return jax.nn.softmax(x, axis=axis)
def _gelu(x):
    return jax.nn.gelu(x, approximate=True)
def _silu(x):
    return jax.nn.silu(x)
def _sigmoid(x):
    return jax.nn.sigmoid(x)
def _layernorm(x, axis=-1, eps=1e-5):
    m = jnp.mean(x, axis=axis, keepdims=True)
    v = jnp.var(x, axis=axis, keepdims=True)
    return (x - m) / jnp.sqrt(v + eps)
def _scatter_add(tgt, idx, src, axis=0):
    return tgt.at[idx].add(src)
def _segment_sum(src, seg, n):
    return jax.ops.segment_sum(src, seg, n)
class _Rng:
    def __init__(self, key):
        self._k = key
    def _next(self):
        self._k, sub = jax.random.split(self._k)
        return sub
    def normal(self, shape):
        return jax.random.normal(self._next(), shape, dtype=jnp.bfloat16)
    def randint(self, lo, hi, shape):
        return jax.random.randint(self._next(), shape, lo, hi, dtype=jnp.int32)
    def uniform(self, shape, lo=0.0, hi=1.0):
        return jax.random.uniform(self._next(), shape, jnp.bfloat16, lo, hi)
    def permutation(self, n):
        return jax.random.permutation(self._next(), n)


kernel_name = 'standalone__self_sup_conv_stem_wavlm__speech'

def setup_inputs():
    _rng = _Rng(jax.random.key(int.from_bytes(__import__("os").urandom(4), "little")))
    _w = (lambda a: (lambda t: t.astype(jnp.bfloat16) if jnp.issubdtype(t.dtype, jnp.floating) else t)(jnp.asarray(a)))
    B, T, D, K = 2, 16000, 512, 31
    scale = (K * D) ** -0.5
    return {
        "x": _w((lambda *s: _rng.normal(s) * 0.05)(B, T, D)),
        "w": _w((lambda *s: _rng.normal(s) * 0.05)(K, D, D) * scale),
        "gn_gamma": _w((lambda *s: _rng.normal(s) * 0.05)(D) * 0.1 + 1.0),
        "gn_beta": _w((lambda *s: _rng.normal(s) * 0.05)(D) * 0.1),
    }

def reference(x, w, gn_gamma, gn_beta):
    B, T, D = x.shape
    K = w.shape[0]
    s = 2
    L = (T - K) // s + 1
    h = jnp.einsum('blc,cd->bld', x[:, 0:s * L:s, :], w[0])
    for i in range(1, K):
        h = h + jnp.einsum('blc,cd->bld', x[:, i:i + s * L:s, :], w[i])
    mu = jnp.einsum('bld->bd', h)[:, None, :] / L
    var = jnp.einsum('bld->bd', (h - mu) ** 2)[:, None, :] / L
    h = (h - mu) / jnp.sqrt(var + 1e-5)
    h = h * gn_gamma[None, None, :] + gn_beta[None, None, :]
    return _gelu(h)
```

```python
import functools
import jax
import jax.numpy as jnp
import jax.experimental.pallas as pl
import jax.experimental.pallas.tpu as pltpu


def _gelu(v):
    c = 0.7978845608028654
    return 0.5 * v * (1.0 + jnp.tanh(c * (v + 0.044715 * (v * v * v))))


def _kernel(x_ref, w_ref, g_ref, b_ref, o_ref, xs_ref, h_ref, s1_ref, s2_ref, *, L, TL, NT, K):
    ph = pl.program_id(1)
    t = pl.program_id(2)
    D = x_ref.shape[-1]
    HT = x_ref.shape[0] // 2

    @pl.when(ph == 0)
    def _():
        @pl.when(t == 0)
        def _():
            s1_ref[...] = jnp.zeros_like(s1_ref)
            s2_ref[...] = jnp.zeros_like(s2_ref)
            xs_ref[pl.ds(HT, xs_ref.shape[0] - HT), :] = jnp.zeros(
                (xs_ref.shape[0] - HT, 2 * D), jnp.float32)

            def body(i, c):
                r = pl.multiple_of(i * 400, 400)
                r2 = pl.multiple_of(i * 200, 200)
                u = pltpu.bitcast(x_ref[pl.ds(r, 400), :], jnp.uint32)
                xs_ref[pl.ds(r2, 200), pl.ds(0, D)] = pltpu.bitcast(u << 16, jnp.float32)
                xs_ref[pl.ds(r2, 200), pl.ds(D, D)] = pltpu.bitcast(
                    u & jnp.uint32(0xFFFF0000), jnp.float32)
                return c
            jax.lax.fori_loop(0, HT // 200, body, 0)

        l0 = pl.multiple_of(t * TL, TL)
        acc = jnp.zeros((TL, D), jnp.float32)
        for j in range((K + 1) // 2):
            lhs = xs_ref[pl.ds(l0 + (j // 8) * 8, TL + 8), :][j % 8:j % 8 + TL].astype(jnp.bfloat16)
            if 2 * j + 1 < K:
                acc += jnp.dot(lhs[:, :D], w_ref[2 * j], preferred_element_type=jnp.float32)
                acc += jnp.dot(lhs[:, D:], w_ref[2 * j + 1], preferred_element_type=jnp.float32)
            else:
                acc += jnp.dot(lhs[:, :D], w_ref[2 * j], preferred_element_type=jnp.float32)
        h_ref[pl.ds(l0, TL), :] = acc
        rows = l0 + jax.lax.broadcasted_iota(jnp.int32, (TL, D), 0)
        am = jnp.where(rows < L, acc, 0.0)
        s1_ref[...] += jnp.sum(am.reshape(TL // 8, 8, D), axis=0)
        s2_ref[...] += jnp.sum((am * am).reshape(TL // 8, 8, D), axis=0)

    @pl.when(ph == 1)
    def _():
        l0 = pl.multiple_of(t * TL, TL)
        mu = jnp.sum(s1_ref[...], axis=0, keepdims=True) * (1.0 / L)
        var = jnp.sum(s2_ref[...], axis=0, keepdims=True) * (1.0 / L) - mu * mu
        var = jnp.maximum(var, 0.0)
        sc = jax.lax.rsqrt(var + 1e-5) * g_ref[...].astype(jnp.float32)
        sh = b_ref[...].astype(jnp.float32) - mu * sc
        o_ref[...] = _gelu(h_ref[pl.ds(l0, TL), :] * sc + sh).astype(o_ref.dtype)


@jax.jit
def pallas_standalone__self_sup_conv_stem_wavlm__speech_kernel(x, w, gn_gamma, gn_beta):
    B, T, D = x.shape
    K = w.shape[0]
    s = 2
    L = (T - K) // s + 1
    TL = 512
    NT = pl.cdiv(L, TL)
    kern = functools.partial(_kernel, L=L, TL=TL, NT=NT, K=K)
    return pl.pallas_call(
        kern,
        grid=(B, 2, NT),
        in_specs=[
            pl.BlockSpec((None, T, D), lambda b, p, t: (b, 0, 0)),
            pl.BlockSpec((K, D, D), lambda b, p, t: (0, 0, 0), pipeline_mode=pl.Buffered(1)),
            pl.BlockSpec((1, D), lambda b, p, t: (0, 0)),
            pl.BlockSpec((1, D), lambda b, p, t: (0, 0)),
        ],
        out_specs=pl.BlockSpec((None, TL, D), lambda b, p, t: (b, t * p, 0)),
        out_shape=jax.ShapeDtypeStruct((B, L, D), x.dtype),
        scratch_shapes=[
            pltpu.VMEM((NT * TL + 16, 2 * D), jnp.float32),
            pltpu.VMEM((NT * TL, D), jnp.float32),
            pltpu.VMEM((8, D), jnp.float32),
            pltpu.VMEM((8, D), jnp.float32),
        ],
        compiler_params=pltpu.CompilerParams(
            dimension_semantics=("arbitrary", "arbitrary", "arbitrary"),
            vmem_limit_bytes=120 * 1024 * 1024,
        ),
    )(x, w, gn_gamma.reshape(1, D), gn_beta.reshape(1, D))
```

```python
import functools
import math

import jax
import jax.numpy as jnp
import jax.experimental.pallas as pl
import jax.experimental.pallas.tpu as pltpu


class _Dag:
    def __init__(self):
        self.nodes = []
        self.memo = {}

    def _node(self, key):
        if key not in self.memo:
            self.memo[key] = len(self.nodes)
            self.nodes.append(key)
        return self.memo[key]

    def inp(self, i, sign=1):
        return (sign, self._node(('in', i)))

    @staticmethod
    def neg(a):
        return None if a is None else (-a[0], a[1])

    def add(self, a, b):
        if a is None:
            return b
        if b is None:
            return a
        (sa, na), (sb, nb) = a, b
        if sa == sb:
            return (sa, self._node(('add', min(na, nb), max(na, nb))))
        if sa > 0:
            return (1, self._node(('sub', na, nb)))
        return (1, self._node(('sub', nb, na)))

    def sub(self, a, b):
        return self.add(a, self.neg(b))

    def mul(self, a, c):
        if a is None or c == 0.0:
            return None
        s, n = a
        c = c * s
        if c == 1.0:
            return (1, n)
        if c == -1.0:
            return (-1, n)
        return (1 if c > 0 else -1, self._node(('mul', n, abs(c))))

    def cadd(self, a, b):
        return (self.add(a[0], b[0]), self.add(a[1], b[1]))

    def csub(self, a, b):
        return (self.sub(a[0], b[0]), self.sub(a[1], b[1]))

    def conj(self, a):
        return (a[0], self.neg(a[1]))

    def cmul_const(self, a, c, s):
        re, im = a
        if re is None or im is None or c == 0.0 or s == 0.0 or abs(c) != abs(s):
            return (self.sub(self.mul(re, c), self.mul(im, s)),
                    self.add(self.mul(re, s), self.mul(im, c)))
        t1 = self.sub(self.mul(re, math.copysign(1, c)), self.mul(im, math.copysign(1, s)))
        t2 = self.add(self.mul(re, math.copysign(1, s)), self.mul(im, math.copysign(1, c)))
        return (self.mul(t1, abs(c)), self.mul(t2, abs(c)))

    @staticmethod
    def tw(k, n):
        k %= n
        if (8 * k) % n == 0:
            r = math.sqrt(0.5)
            return [(1.0, 0.0), (r, -r), (0.0, -1.0), (-r, -r),
                    (-1.0, 0.0), (-r, r), (0.0, 1.0), (r, r)][8 * k // n]
        return (math.cos(2 * math.pi * k / n), -math.sin(2 * math.pi * k / n))

    def rfft_combine(self, e, o1, o3, n, emit_bin=None):
        q = n // 4
        out = [None] * (n // 2 + 1)

        def E(k):
            return e[k] if k <= q else self.conj(e[n // 2 - k])

        def done(*ks):
            if emit_bin is not None:
                for kk in ks:
                    emit_bin(kk, out)
        s0 = self.add(o1[0][0], o3[0][0])
        d0 = self.sub(o1[0][0], o3[0][0])
        out[0] = (self.add(e[0][0], s0), None)
        out[n // 2] = (self.sub(e[0][0], s0), None)
        out[q] = (e[q][0], self.neg(d0))
        done(0, n // 2, q)
        for k in range(1, q // 2 + 1):
            if 2 * k == q:
                a1, a3 = o1[k][0], o3[k][0]
                r = math.sqrt(0.5)
                S = (self.mul(self.sub(a1, a3), r), self.neg(self.mul(self.add(a1, a3), r)))
                out[k] = self.cadd(E(k), S)
                out[n // 2 - k] = self.conj(self.csub(E(k), S))
                done(k, n // 2 - k)
                continue
            z1 = self.cmul_const(o1[k], *self.tw(k, n))
            z3 = self.cmul_const(o3[k], *self.tw(3 * k, n))
            S = self.cadd(z1, z3)
            Dd = self.csub(z1, z3)
            mi_d = (Dd[1], self.neg(Dd[0]))
            out[k] = self.cadd(E(k), S)
            out[n // 2 - k] = self.conj(self.csub(E(k), S))
            out[q + k] = self.cadd(E(q + k), mi_d)
            out[q - k] = self.conj(self.csub(E(q + k), mi_d))
            done(k, n // 2 - k, q + k, q - k)
        return out

    def rfft(self, x):
        n = len(x)
        if n == 1:
            return [(x[0], None)]
        if n == 2:
            return [(self.add(x[0], x[1]), None), (self.sub(x[0], x[1]), None)]
        e = self.rfft(x[0::2])
        o1 = self.rfft(x[1::4])
        o3 = self.rfft(x[3::4])
        return self.rfft_combine(e, o1, o3, n)

    def irfft_split(self, X):
        n = 2 * (len(X) - 1)
        q, h = n // 4, n // 2
        U = [None] * (q + 1)
        z1 = [None] * (n // 8 + 1)
        z3 = [None] * (n // 8 + 1)
        U[0] = (self.add(X[0][0], X[h][0]), None)
        U[q] = (self.mul(X[q][0], 2.0), None)
        a0 = self.sub(X[0][0], X[h][0])
        ib0 = self.neg(self.mul(X[q][1], 2.0))
        z1[0] = (self.add(a0, ib0), None)
        z3[0] = (self.sub(a0, ib0), None)
        for k in range(1, n // 8 + 1):
            U[k] = self.cadd(X[k], self.conj(X[h - k]))
            A = self.csub(X[k], self.conj(X[h - k]))
            if 8 * k == n:
                r2 = math.sqrt(2.0)
                z1[k] = (self.mul(self.sub(A[0], A[1]), r2), None)
                z3[k] = (self.mul(self.add(A[0], A[1]), -r2), None)
                continue
            U[q - k] = self.cadd(X[q - k], self.conj(X[q + k]))
            Bk = self.csub(X[q + k], self.conj(X[q - k]))
            iB = (self.neg(Bk[1]), Bk[0])
            z1[k] = self.cmul_const(self.cadd(A, iB), *self.tw(-k, n))
            z3[k] = self.cmul_const(self.csub(A, iB), *self.tw(-3 * k, n))
        return U, z1, z3

    def irfft(self, X):
        if len(X) == 1:
            return [X[0][0]]
        if len(X) == 2:
            return [self.add(X[0][0], X[1][0]), self.sub(X[0][0], X[1][0])]
        n = 2 * (len(X) - 1)
        if n == 4:
            U = [(self.add(X[0][0], X[2][0]), None), (self.mul(X[1][0], 2.0), None)]
            a0 = self.sub(X[0][0], X[2][0])
            ib0 = self.neg(self.mul(X[1][1], 2.0))
            z1 = [(self.add(a0, ib0), None)]
            z3 = [(self.sub(a0, ib0), None)]
        else:
            U, z1, z3 = self.irfft_split(X)
        out = [None] * n
        out[0::2] = self.irfft(U)
        out[1::4] = self.irfft(z1)
        out[3::4] = self.irfft(z3)
        return out

    def emit(self, outs, load, store=None, zero=None):
        nodes = self.nodes
        uses = {}
        need = set()
        stack = [o[1] for o in outs if o is not None]
        while stack:
            t = stack.pop()
            if t in need:
                continue
            need.add(t)
            key = nodes[t]
            if key[0] != 'in':
                for d in (key[1:3] if key[0] != 'mul' else key[1:2]):
                    uses[d] = uses.get(d, 0) + 1
                    stack.append(d)
        by_node = {}
        for i, o in enumerate(outs):
            if o is not None:
                by_node.setdefault(o[1], []).append((i, o[0]))
        val = {}
        res = [None] * len(outs)

        def get(t):
            if t not in val:
                val[t] = load(nodes[t][1])
            return val[t]

        def put(i, v):
            if store is not None:
                store(i, v)
            else:
                res[i] = v

        def fin(t, flipped):
            for i, sg in by_node.get(t, ()):
                put(i, val[t] if (sg > 0) != flipped else -val[t])
        for t, key in enumerate(nodes):
            if t not in need or key[0] == 'in':
                continue
            flipped = False
            if key[0] == 'add':
                val[t] = get(key[1]) + get(key[2])
            elif key[0] == 'sub':
                if uses.get(t, 0) == 0 and all(sg < 0 for _, sg in by_node[t]):
                    flipped = True
                    first, second = get(key[1]), get(key[2])
                    val[t] = second - first
                else:
                    val[t] = get(key[1]) - get(key[2])
            else:
                if uses.get(t, 0) == 0 and all(sg < 0 for _, sg in by_node[t]):
                    flipped = True
                    val[t] = get(key[1]) * (-key[2])
                else:
                    val[t] = get(key[1]) * key[2]
            fin(t, flipped)
        for i, o in enumerate(outs):
            if o is None:
                put(i, zero())
            elif nodes[o[1]][0] == 'in':
                v = get(o[1])
                put(i, v if o[0] > 0 else -v)
        return res


def _spec_flat(X):
    n2 = len(X) - 1
    return [X[0][0], X[n2][0]] + [v for k in range(1, n2) for v in X[k]]


def _spec_in(g, base, n, src=None):
    def one(i):
        if src is None:
            return g.inp(base + i)
        if src[i] is None:
            return None
        return g.inp(base + src[i][1], src[i][0])
    return ([(one(0), None)] + [(one(2 * k), one(2 * k + 1)) for k in range(1, n // 2)] + [(one(1), None)])


def _unsigned(outs):
    slot, raw, src = {}, [], []
    for o in outs:
        if o is None:
            src.append(None)
            continue
        if o[1] not in slot:
            slot[o[1]] = len(raw)
            raw.append((1, o[1]))
        src.append((o[0], slot[o[1]]))
    return raw, src


def _sub_rfft(n, taps=None):
    g = _Dag()
    X = g.rfft([g.inp(i) if taps is None or i < taps else None for i in range(n)])
    raw, src = _unsigned(_spec_flat(X))
    return g, raw, src


def _combine(N, weights, srcs, flips=None):
    g = _Dag()
    e = _spec_in(g, 0, N // 2, srcs[0])
    o1 = _spec_in(g, N // 2, N // 4, srcs[1])
    o3 = _spec_in(g, 3 * N // 4, N // 4, srcs[2])
    outs = [None] * (3 * (N // 2) - 1)

    def emit_bin(k, out):
        a, b = out[k]
        if k == 0:
            outs[0] = a
        elif k == N // 2:
            outs[1] = a
        elif weights:
            outs[3 * k - 1:3 * k + 2] = [g.sub(a, b), b, a]
        else:
            outs[3 * k - 1:3 * k + 2] = [a, g.add(a, b), g.sub(b, a)]
    g.rfft_combine(e, o1, o3, N, emit_bin)
    return g, outs


def _inv_split(N, src):
    g = _Dag()
    U, z1, z3 = g.irfft_split(_spec_in(g, 0, N, src))
    return g, _spec_flat(U), _spec_flat(z1), _spec_flat(z3)


def _sub_irfft(n, keep, src):
    g = _Dag()
    y = g.irfft(_spec_in(g, 0, n, src))
    return g, y[:keep]


def _flippable(g, outs):
    used = set()
    for key in g.nodes:
        if key[0] != 'in':
            used.update(key[1:3] if key[0] != 'mul' else key[1:2])
    cnt = {}
    for o in outs:
        cnt[o[1]] = cnt.get(o[1], 0) + 1
    return [g.nodes[o[1]][0] in ('sub', 'mul') and o[1] not in used and cnt[o[1]] == 1 for o in outs]


def _balance_signs(gx, ox, gw, ow, N, force=None):
    fx = _flippable(gx, ox)
    ox = list(ox)
    sig = []
    for k in range(N // 2):
        idx = [0] if k == 0 else [3 * k - 1, 3 * k, 3 * k + 1]
        if k == 0:
            s01 = (ox[0][0] * ow[0][0], ox[1][0] * ow[1][0]) if force is None else force[0]
            ox[0] = (ox[0][0] * ow[0][0] * s01[0], ox[0][1])
            ox[1] = (ox[1][0] * ow[1][0] * s01[1], ox[1][1])
            sig.append(s01)
            continue
        p = [ox[i][0] * ow[i][0] for i in idx]
        best = None
        for s in (1, -1):
            cost = sum(0 if (pi == s or fx[i]) else 1 for pi, i in zip(p, idx))
            if best is None or cost < best[0]:
                best = (cost, s)
        s = best[1] if force is None else force[k][0]
        for pi, i in zip(p, idx):
            ox[i] = (1 if pi == s else -1, ox[i][1])
        sig.append((s, s))
    return ox, sig


N_FFT = 64
HOP = 49
NMAT = 95
HI16 = 0xFFFF0000


def _f32(u):
    return pltpu.bitcast(u, jnp.float32)


def _half(u, p):
    return _f32(u << 16) if p == 0 else _f32(u & jnp.uint32(HI16))


def _pack(a, b):
    return pltpu.pack_elementwise([a, b], packed_dtype=jnp.bfloat16)


@functools.lru_cache(maxsize=None)
def _codelets():
    N = N_FFT
    c = {}
    c['x32'] = _sub_rfft(32)
    c['x16'] = _sub_rfft(16)
    gx, ox = _combine(N, False, (c['x32'][2], c['x16'][2], c['x16'][2]))
    sig = None
    for p, taps in ((0, 16), (1, 15)):
        e = _sub_rfft(32, (taps + 1) // 2)
        o1 = _sub_rfft(16, (taps + 2) // 4)
        o3 = _sub_rfft(16, taps // 4)
        gw, ow = _combine(N, True, (e[2], o1[2], o3[2]))
        oxp, sig = _balance_signs(gx, ox, gw, ow, N, sig)
        c['w', p] = (e, o1, o3, gw, [(1, o[1]) for o in ow])
        c['xc', p] = (gx, oxp)
    src = [(sig[0][0], 0), (sig[0][1], 1)] + [(sig[k][0], 2 * k + t) for k in range(1, N // 2) for t in range(2)]
    gi, oU, o1, o3 = _inv_split(N, src)
    rU, sU = _unsigned(oU)
    r1, s1 = _unsigned(o1)
    r3, s3 = _unsigned(o3)
    assert (len(rU), len(r1), len(r3)) == (32, 16, 16)
    c['inv'] = (gi, rU + r1 + r3)
    c['iu'] = _sub_irfft(32, (HOP + 1) // 2, sU)
    c['i1'] = _sub_irfft(16, (HOP + 2) // 4, s1)
    c['i3'] = _sub_irfft(16, HOP // 4, s3)
    return c


def _two_half_fft(ld, st, out, subs, comb):
    (ge, oe, _), (g1, o1, _), (g3, o3, _) = subs

    def stage(base):
        def f(i, v):
            st[base + i] = v
        return f
    ge.emit(oe, lambda i: ld(0, 2 * i), store=stage(0))
    g1.emit(o1, lambda i: ld(0, 4 * i + 1), store=stage(32))
    g3.emit(o3, lambda i: ld(0, 4 * i + 3), store=stage(48))
    ge.emit(oe, lambda i: ld(1, 2 * i), store=stage(64))
    r1 = g1.emit(o1, lambda i: ld(1, 4 * i + 1))
    r3 = g3.emit(o3, lambda i: ld(1, 4 * i + 3))

    def ldc(i):
        if i < 32:
            b = st[64 + i]
        elif i < 48:
            b = r1[i - 32]
        else:
            b = r3[i - 48]
        return jnp.concatenate([st[i], b], axis=0)
    comb[0].emit(comb[1], ldc, store=lambda i, v: out(i, _pack(v[:8], v[8:])))


def _kernel(x_hbm, w_hbm, g_ref, b_ref, o_hbm,
            xbuf, wbuf, xh, wh, acc, stx, stw, obuf, sem_x, sem_w, sem_o,
            *, B, T, D, K, L, RB):
    cod = _codelets()
    R = B * RB
    NG = R // 16
    NJ = D // 128
    XB = RB * HOP
    TH = T // 2

    def x_copies(j, slot):
        xv = xbuf.bitcast(jnp.bfloat16)
        return [pltpu.make_async_copy(
            x_hbm.at[b, :, pl.ds(j * 128, 128)],
            xv.at[slot, pl.ds(2 * b * XB, T), :], sem_x.at[slot, b]) for b in range(B)]

    def w_copy(j, slot):
        return pltpu.make_async_copy(
            w_hbm.at[:, pl.ds(j * 128, 128), :], wbuf.bitcast(jnp.bfloat16).at[slot], sem_w.at[slot])

    def start_in(j, slot):
        w_copy(j, slot).start()
        for c in x_copies(j, slot):
            c.start()

    def wait_in(j, slot):
        w_copy(j, slot).wait()
        for c in x_copies(j, slot):
            c.wait()

    start_in(0, 0)
    start_in(1, 1)

    def zero_acc(i, c):
        acc[i] = jnp.zeros(acc.shape[1:], jnp.float32)
        return c
    jax.lax.fori_loop(0, acc.shape[0], zero_acc, 0)
    for slot in range(2):
        for b in range(B):
            hi = (b + 1) * XB if b + 1 < B else xbuf.shape[1]
            xbuf[slot, pl.ds(b * XB + TH, hi - b * XB - TH), :] = jnp.zeros((hi - b * XB - TH, 128), jnp.uint32)

    def x_fft(G, p, xslot, so):
        def ld(e, n):
            return _half(xbuf[xslot, pl.ds(G * (16 * HOP) + HOP * e + n, 8, stride=2 * HOP), :], p)

        def out(i, v):
            xh[so, i, pl.ds(pl.multiple_of(G * 8, 8), 8), :] = v
        _two_half_fft(ld, stx, out, (cod['x32'], cod['x16'], cod['x16']), cod['xc', p])

    def w_fft(t, p, wslot, so):
        rs = pl.ds(pl.multiple_of((t // NJ) * 8, 8), 8)
        cs = pl.ds(pl.multiple_of((t % NJ) * 128, 128), 128)

        def ld(e, j):
            return _half(wbuf[wslot, 2 * j + p, rs, cs], e)

        def out(i, v):
            wh[so, i, rs, cs] = v
        e, o1, o3, gw, ow = cod['w', p]
        _two_half_fft(ld, stw, out, (e, o1, o3), (gw, ow))

    def dot(si, i):
        a = pltpu.bitcast(xh[si, i], jnp.bfloat16)
        b = pltpu.bitcast(wh[si, i], jnp.bfloat16)
        return jnp.dot(a, b, preferred_element_type=jnp.float32)

    def mm_bin(k, si):
        r0 = dot(si, 3 * k - 1)
        r1 = dot(si, 3 * k)
        r2 = dot(si, 3 * k + 1)
        acc[2 * k] = acc[2 * k] + (r0 + r1)
        acc[2 * k + 1] = acc[2 * k + 1] + (r0 + r2)

    def mm_real(si):
        acc[0] = acc[0] + dot(si, 0)
        acc[1] = acc[1] + dot(si, 1)

    NW = 8 * NJ

    def chunk(si, nxt):
        mm_real(si)
        if nxt is None:
            def body(i, c):
                for u in range(5):
                    mm_bin(1 + 5 * i + u, si)
                return c
            jax.lax.fori_loop(0, 6, body, 0)
            mm_bin(N_FFT // 2 - 1, si)
            return
        p, islot = nxt
        w_fft(0, p, islot, 1 - si)

        def body_a(i, c):
            mm_bin(1 + i, si)
            x_fft(i, p, islot, 1 - si)
            w_fft(1 + i, p, islot, 1 - si)
            return c
        jax.lax.fori_loop(0, NG, body_a, 0)

        def body_b(i, c):
            mm_bin(1 + i, si)
            w_fft(1 + i, p, islot, 1 - si)
            return c
        jax.lax.fori_loop(NG, NW - 1, body_b, 0)

    wait_in(0, 0)

    def pro_w(t, c):
        w_fft(t, 0, 0, 0)
        return c
    jax.lax.fori_loop(0, NW, pro_w, 0)

    def pro_x(G, c):
        x_fft(G, 0, 0, 0)
        return c
    jax.lax.fori_loop(0, NG, pro_x, 0)

    def jstep(j, c):
        islot = j % 2
        chunk(0, (1, islot))
        wait_in(j + 1, 1 - islot)

        @pl.when(j + 2 < NJ)
        def _():
            start_in(j + 2, islot)
        chunk(1, (0, 1 - islot))
        return c
    jax.lax.fori_loop(0, NJ - 1, jstep, 0)
    chunk(0, (1, (NJ - 1) % 2))
    chunk(1, None)

    GB = RB // 8
    gi, oi = cod['inv']

    def y_fft(g8, j, mask_from):
        rs = pl.ds(pl.multiple_of(g8 * 8, 8), 8)
        cs = pl.ds(pl.multiple_of(j * 128, 128), 128)
        kept = {}

        def st1(i, v):
            if i < 32:
                stx[i] = v
            else:
                kept[i] = v
        gi.emit(oi, lambda i: acc[i, rs, cs], store=st1)
        s = [None, None]

        def fin(n, v):
            acc[n, rs, cs] = v
            if mask_from is not None:
                wrow = jax.lax.broadcasted_iota(jnp.int32, (8, 128), 0)
                v = jnp.where(wrow * HOP + n < mask_from, v, 0.0)
            s[0] = v if s[0] is None else s[0] + v
            s[1] = v * v if s[1] is None else s[1] + v * v
        cod['i1'][0].emit(cod['i1'][1], lambda i: kept[32 + i], store=lambda i, v: fin(4 * i + 1, v))
        cod['i3'][0].emit(cod['i3'][1], lambda i: kept[48 + i], store=lambda i, v: fin(4 * i + 3, v))
        cod['iu'][0].emit(cod['iu'][1], lambda i: stx[i], store=lambda i, v: fin(2 * i, v))
        return s

    def stats_body(b):
        def body(t, c):
            g = t // NJ
            j = t % NJ
            s1, s2 = y_fft(b * GB + g, j, None)
            cs = pl.ds(pl.multiple_of(j * 128, 128), 128)
            stw[2 * b * NJ + j] = stw[2 * b * NJ + j] + s1
            stw[(2 * b + 1) * NJ + j] = stw[(2 * b + 1) * NJ + j] + s2
            return c
        return body
    for i in range(2 * B * NJ):
        stw[i] = jnp.zeros((8, 128), jnp.float32)
    nfull = (L // HOP) // 8
    for b in range(B):
        jax.lax.fori_loop(0, nfull * NJ, stats_body(b), 0)
        for g in range(nfull, GB):
            def tail(j, c, b=b, g=g):
                s1, s2 = y_fft(b * GB + g, j, L - g * 8 * HOP)
                stw[2 * b * NJ + j] = stw[2 * b * NJ + j] + s1
                stw[(2 * b + 1) * NJ + j] = stw[(2 * b + 1) * NJ + j] + s2
                return c
            jax.lax.fori_loop(0, NJ, tail, 0)

    inv_n = 1.0 / N_FFT
    for b in range(B):
        for j in range(NJ):
            cs = pl.ds(j * 128, 128)
            s1 = jnp.sum(stw[2 * b * NJ + j], axis=0, keepdims=True) * (inv_n / L)
            s2 = jnp.sum(stw[(2 * b + 1) * NJ + j], axis=0, keepdims=True) * (inv_n * inv_n / L)
            var = jnp.maximum(s2 - s1 * s1, 0.0)
            rstd = jax.lax.rsqrt(var + 1e-5)
            gam = g_ref[:, cs].astype(jnp.float32)
            bet = b_ref[:, cs].astype(jnp.float32)
            sc = rstd * gam
            stw[2 * b * NJ + j] = jnp.broadcast_to(sc * (0.5 * inv_n), (8, 128))
            stw[(2 * b + 1) * NJ + j] = jnp.broadcast_to((bet - s1 * sc) * 0.5, (8, 128))

    c0 = 2.0 * 0.7978845608028654
    c1 = 8.0 * 0.7978845608028654 * 0.044715
    GL = 8 * HOP
    ov = obuf.bitcast(jnp.bfloat16)

    def out_copy(g, slot, rows):
        return pltpu.make_async_copy(
            ov.at[slot, pl.ds(0, rows * 2 * NJ), :], o_hbm.at[pl.ds(g * (GL * 2 * NJ), rows * 2 * NJ), :],
            sem_o.at[slot])

    def fill(g, slot):
        def body(j, c):
            cs = pl.ds(pl.multiple_of(j * 128, 128), 128)
            par = [(stw[2 * b * NJ + j], stw[(2 * b + 1) * NJ + j]) for b in range(B)]
            for n in range(HOP):
                r = []
                for b in range(B):
                    h = acc[n, pl.ds(pl.multiple_of((b * GB + g) * 8, 8), 8), cs]
                    y = h * par[b][0] + par[b][1]
                    z = ((y * y) * c1 + c0) * y
                    r.append(y * jnp.tanh(z) + y)
                obuf[slot, pl.ds(n * NJ + j, 8, stride=HOP * NJ), :] = _pack(r[0], r[1])
            return c
        jax.lax.fori_loop(0, NJ, body, 0)

    ngo = pl.cdiv(L, GL)
    nfo = L // GL

    def out_body(g, c):
        slot = g % 2

        @pl.when(g >= 2)
        def _():
            out_copy(g - 2, slot, GL).wait()
        fill(g, slot)
        out_copy(g, slot, GL).start()
        return c
    jax.lax.fori_loop(0, nfo, out_body, 0)
    pend = [(g, GL) for g in range(max(nfo - 2, 0), nfo)]
    for g in range(nfo, ngo):
        slot = g % 2
        for pg in [q for q in pend if q[0] % 2 == slot]:
            out_copy(pg[0], slot, pg[1]).wait()
            pend.remove(pg)
        fill(g, slot)
        out_copy(g, slot, L - g * GL).start()
        pend.append((g, L - g * GL))
    for g, rows in pend:
        out_copy(g, g % 2, rows).wait()


@jax.jit
def pallas_standalone__self_sup_conv_stem_wavlm__speech_kernel(x, w, gn_gamma, gn_beta):
    B, T, D = x.shape
    K = w.shape[0]
    s = 2
    L = (T - K) // s + 1
    assert B == 2 and K == 31 and D % 128 == 0 and T % 16 == 0
    nwin = pl.cdiv(L, HOP)
    RB = pl.cdiv(nwin, 8) * 8
    R = B * RB
    NJ = D // 128
    xrows = pl.cdiv(R * HOP + N_FFT, 8) * 8
    kern = functools.partial(_kernel, B=B, T=T, D=D, K=K, L=L, RB=RB)
    out = pl.pallas_call(
        kern,
        in_specs=[
            pl.BlockSpec(memory_space=pl.ANY),
            pl.BlockSpec(memory_space=pl.ANY),
            pl.BlockSpec(memory_space=pltpu.VMEM),
            pl.BlockSpec(memory_space=pltpu.VMEM),
        ],
        out_specs=pl.BlockSpec(memory_space=pl.ANY),
        out_shape=jax.ShapeDtypeStruct((L * NJ * B, 128), x.dtype),
        scratch_shapes=[
            pltpu.VMEM((2, xrows, 128), jnp.uint32),
            pltpu.VMEM((2, K, 64, D), jnp.uint32),
            pltpu.VMEM((2, NMAT, R // 2, 128), jnp.uint32),
            pltpu.VMEM((2, NMAT, 64, D), jnp.uint32),
            pltpu.VMEM((N_FFT, R, D), jnp.float32),
            pltpu.VMEM((96, 8, 128), jnp.float32),
            pltpu.VMEM((96, 8, 128), jnp.float32),
            pltpu.VMEM((2, 8 * HOP * NJ, 128), jnp.uint32),
            pltpu.SemaphoreType.DMA((2, B)),
            pltpu.SemaphoreType.DMA((2,)),
            pltpu.SemaphoreType.DMA((2,)),
        ],
        compiler_params=pltpu.CompilerParams(vmem_limit_bytes=124 * 1024 * 1024),
    )(x, w, gn_gamma.reshape(1, D), gn_beta.reshape(1, D))
    return jnp.transpose(out.reshape(L, NJ, B, 128), (2, 0, 1, 3)).reshape(B, L, D)
```

```python
import functools
import math

import jax
import jax.numpy as jnp
import jax.experimental.pallas as pl
import jax.experimental.pallas.tpu as pltpu


class _Dag:
    def __init__(self):
        self.nodes = []
        self.memo = {}

    def _node(self, key):
        if key not in self.memo:
            self.memo[key] = len(self.nodes)
            self.nodes.append(key)
        return self.memo[key]

    def inp(self, i, sign=1):
        return (sign, self._node(('in', i)))

    @staticmethod
    def neg(a):
        return None if a is None else (-a[0], a[1])

    def add(self, a, b):
        if a is None:
            return b
        if b is None:
            return a
        (sa, na), (sb, nb) = a, b
        if sa == sb:
            return (sa, self._node(('add', min(na, nb), max(na, nb))))
        if sa > 0:
            return (1, self._node(('sub', na, nb)))
        return (1, self._node(('sub', nb, na)))

    def sub(self, a, b):
        return self.add(a, self.neg(b))

    def mul(self, a, c):
        if a is None or c == 0.0:
            return None
        s, n = a
        c = c * s
        if c == 1.0:
            return (1, n)
        if c == -1.0:
            return (-1, n)
        return (1 if c > 0 else -1, self._node(('mul', n, abs(c))))

    def cadd(self, a, b):
        return (self.add(a[0], b[0]), self.add(a[1], b[1]))

    def csub(self, a, b):
        return (self.sub(a[0], b[0]), self.sub(a[1], b[1]))

    def conj(self, a):
        return (a[0], self.neg(a[1]))

    def cmul_const(self, a, c, s):
        re, im = a
        if re is None or im is None or c == 0.0 or s == 0.0 or abs(c) != abs(s):
            return (self.sub(self.mul(re, c), self.mul(im, s)),
                    self.add(self.mul(re, s), self.mul(im, c)))
        t1 = self.sub(self.mul(re, math.copysign(1, c)), self.mul(im, math.copysign(1, s)))
        t2 = self.add(self.mul(re, math.copysign(1, s)), self.mul(im, math.copysign(1, c)))
        return (self.mul(t1, abs(c)), self.mul(t2, abs(c)))

    @staticmethod
    def tw(k, n):
        k %= n
        if (8 * k) % n == 0:
            r = math.sqrt(0.5)
            return [(1.0, 0.0), (r, -r), (0.0, -1.0), (-r, -r),
                    (-1.0, 0.0), (-r, r), (0.0, 1.0), (r, r)][8 * k // n]
        return (math.cos(2 * math.pi * k / n), -math.sin(2 * math.pi * k / n))

    def rfft_combine(self, e, o1, o3, n, emit_bin=None):
        q = n // 4
        out = [None] * (n // 2 + 1)

        def E(k):
            return e[k] if k <= q else self.conj(e[n // 2 - k])

        def done(*ks):
            if emit_bin is not None:
                for kk in ks:
                    emit_bin(kk, out)
        s0 = self.add(o1[0][0], o3[0][0])
        d0 = self.sub(o1[0][0], o3[0][0])
        out[0] = (self.add(e[0][0], s0), None)
        out[n // 2] = (self.sub(e[0][0], s0), None)
        out[q] = (e[q][0], self.neg(d0))
        done(0, n // 2, q)
        for k in range(1, q // 2 + 1):
            if 2 * k == q:
                a1, a3 = o1[k][0], o3[k][0]
                r = math.sqrt(0.5)
                S = (self.mul(self.sub(a1, a3), r), self.neg(self.mul(self.add(a1, a3), r)))
                out[k] = self.cadd(E(k), S)
                out[n // 2 - k] = self.conj(self.csub(E(k), S))
                done(k, n // 2 - k)
                continue
            z1 = self.cmul_const(o1[k], *self.tw(k, n))
            z3 = self.cmul_const(o3[k], *self.tw(3 * k, n))
            S = self.cadd(z1, z3)
            Dd = self.csub(z1, z3)
            mi_d = (Dd[1], self.neg(Dd[0]))
            out[k] = self.cadd(E(k), S)
            out[n // 2 - k] = self.conj(self.csub(E(k), S))
            out[q + k] = self.cadd(E(q + k), mi_d)
            out[q - k] = self.conj(self.csub(E(q + k), mi_d))
            done(k, n // 2 - k, q + k, q - k)
        return out

    def rfft(self, x):
        n = len(x)
        if n == 1:
            return [(x[0], None)]
        if n == 2:
            return [(self.add(x[0], x[1]), None), (self.sub(x[0], x[1]), None)]
        e = self.rfft(x[0::2])
        o1 = self.rfft(x[1::4])
        o3 = self.rfft(x[3::4])
        return self.rfft_combine(e, o1, o3, n)

    def irfft_split(self, X):
        n = 2 * (len(X) - 1)
        q, h = n // 4, n // 2
        U = [None] * (q + 1)
        z1 = [None] * (n // 8 + 1)
        z3 = [None] * (n // 8 + 1)
        U[0] = (self.add(X[0][0], X[h][0]), None)
        U[q] = (self.mul(X[q][0], 2.0), None)
        a0 = self.sub(X[0][0], X[h][0])
        ib0 = self.neg(self.mul(X[q][1], 2.0))
        z1[0] = (self.add(a0, ib0), None)
        z3[0] = (self.sub(a0, ib0), None)
        for k in range(1, n // 8 + 1):
            U[k] = self.cadd(X[k], self.conj(X[h - k]))
            A = self.csub(X[k], self.conj(X[h - k]))
            if 8 * k == n:
                r2 = math.sqrt(2.0)
                z1[k] = (self.mul(self.sub(A[0], A[1]), r2), None)
                z3[k] = (self.mul(self.add(A[0], A[1]), -r2), None)
                continue
            U[q - k] = self.cadd(X[q - k], self.conj(X[q + k]))
            Bk = self.csub(X[q + k], self.conj(X[q - k]))
            iB = (self.neg(Bk[1]), Bk[0])
            z1[k] = self.cmul_const(self.cadd(A, iB), *self.tw(-k, n))
            z3[k] = self.cmul_const(self.csub(A, iB), *self.tw(-3 * k, n))
        return U, z1, z3

    def irfft(self, X):
        if len(X) == 1:
            return [X[0][0]]
        if len(X) == 2:
            return [self.add(X[0][0], X[1][0]), self.sub(X[0][0], X[1][0])]
        n = 2 * (len(X) - 1)
        if n == 4:
            U = [(self.add(X[0][0], X[2][0]), None), (self.mul(X[1][0], 2.0), None)]
            a0 = self.sub(X[0][0], X[2][0])
            ib0 = self.neg(self.mul(X[1][1], 2.0))
            z1 = [(self.add(a0, ib0), None)]
            z3 = [(self.sub(a0, ib0), None)]
        else:
            U, z1, z3 = self.irfft_split(X)
        out = [None] * n
        out[0::2] = self.irfft(U)
        out[1::4] = self.irfft(z1)
        out[3::4] = self.irfft(z3)
        return out

    def emit(self, outs, load, store=None, zero=None):
        nodes = self.nodes
        uses = {}
        need = set()
        stack = [o[1] for o in outs if o is not None]
        while stack:
            t = stack.pop()
            if t in need:
                continue
            need.add(t)
            key = nodes[t]
            if key[0] != 'in':
                for d in (key[1:3] if key[0] != 'mul' else key[1:2]):
                    uses[d] = uses.get(d, 0) + 1
                    stack.append(d)
        by_node = {}
        for i, o in enumerate(outs):
            if o is not None:
                by_node.setdefault(o[1], []).append((i, o[0]))
        val = {}
        res = [None] * len(outs)

        def get(t):
            if t not in val:
                val[t] = load(nodes[t][1])
            return val[t]

        def put(i, v):
            if store is not None:
                store(i, v)
            else:
                res[i] = v

        def fin(t, flipped):
            for i, sg in by_node.get(t, ()):
                put(i, val[t] if (sg > 0) != flipped else -val[t])
        for t, key in enumerate(nodes):
            if t not in need or key[0] == 'in':
                continue
            flipped = False
            if key[0] == 'add':
                val[t] = get(key[1]) + get(key[2])
            elif key[0] == 'sub':
                if uses.get(t, 0) == 0 and all(sg < 0 for _, sg in by_node[t]):
                    flipped = True
                    first, second = get(key[1]), get(key[2])
                    val[t] = second - first
                else:
                    val[t] = get(key[1]) - get(key[2])
            else:
                if uses.get(t, 0) == 0 and all(sg < 0 for _, sg in by_node[t]):
                    flipped = True
                    val[t] = get(key[1]) * (-key[2])
                else:
                    val[t] = get(key[1]) * key[2]
            fin(t, flipped)
        for i, o in enumerate(outs):
            if o is None:
                put(i, zero())
            elif nodes[o[1]][0] == 'in':
                v = get(o[1])
                put(i, v if o[0] > 0 else -v)
        return res


def _spec_flat(X):
    n2 = len(X) - 1
    return [X[0][0], X[n2][0]] + [v for k in range(1, n2) for v in X[k]]


def _spec_in(g, base, n, src=None):
    def one(i):
        if src is None:
            return g.inp(base + i)
        if src[i] is None:
            return None
        return g.inp(base + src[i][1], src[i][0])
    return ([(one(0), None)] + [(one(2 * k), one(2 * k + 1)) for k in range(1, n // 2)] + [(one(1), None)])


def _unsigned(outs):
    slot, raw, src = {}, [], []
    for o in outs:
        if o is None:
            src.append(None)
            continue
        if o[1] not in slot:
            slot[o[1]] = len(raw)
            raw.append((1, o[1]))
        src.append((o[0], slot[o[1]]))
    return raw, src


def _sub_rfft(n, taps=None):
    g = _Dag()
    X = g.rfft([g.inp(i) if taps is None or i < taps else None for i in range(n)])
    raw, src = _unsigned(_spec_flat(X))
    return g, raw, src


def _combine(N, weights, srcs, flips=None):
    g = _Dag()
    e = _spec_in(g, 0, N // 2, srcs[0])
    o1 = _spec_in(g, N // 2, N // 4, srcs[1])
    o3 = _spec_in(g, 3 * N // 4, N // 4, srcs[2])
    outs = [None] * (3 * (N // 2) - 1)

    def emit_bin(k, out):
        a, b = out[k]
        if k == 0:
            outs[0] = a
        elif k == N // 2:
            outs[1] = a
        elif weights:
            outs[3 * k - 1:3 * k + 2] = [g.sub(a, b), b, a]
        else:
            outs[3 * k - 1:3 * k + 2] = [a, g.add(a, b), g.sub(b, a)]
    g.rfft_combine(e, o1, o3, N, emit_bin)
    return g, outs


def _inv_split(N, src):
    g = _Dag()
    U, z1, z3 = g.irfft_split(_spec_in(g, 0, N, src))
    return g, _spec_flat(U), _spec_flat(z1), _spec_flat(z3)


def _sub_irfft(n, keep, src):
    g = _Dag()
    y = g.irfft(_spec_in(g, 0, n, src))
    return g, y[:keep]


def _flippable(g, outs):
    used = set()
    for key in g.nodes:
        if key[0] != 'in':
            used.update(key[1:3] if key[0] != 'mul' else key[1:2])
    cnt = {}
    for o in outs:
        cnt[o[1]] = cnt.get(o[1], 0) + 1
    return [g.nodes[o[1]][0] in ('sub', 'mul') and o[1] not in used and cnt[o[1]] == 1 for o in outs]


def _balance_signs(gx, ox, gw, ow, N, force=None):
    fx = _flippable(gx, ox)
    ox = list(ox)
    sig = []
    for k in range(N // 2):
        idx = [0] if k == 0 else [3 * k - 1, 3 * k, 3 * k + 1]
        if k == 0:
            s01 = (ox[0][0] * ow[0][0], ox[1][0] * ow[1][0]) if force is None else force[0]
            ox[0] = (ox[0][0] * ow[0][0] * s01[0], ox[0][1])
            ox[1] = (ox[1][0] * ow[1][0] * s01[1], ox[1][1])
            sig.append(s01)
            continue
        p = [ox[i][0] * ow[i][0] for i in idx]
        best = None
        for s in (1, -1):
            cost = sum(0 if (pi == s or fx[i]) else 1 for pi, i in zip(p, idx))
            if best is None or cost < best[0]:
                best = (cost, s)
        s = best[1] if force is None else force[k][0]
        for pi, i in zip(p, idx):
            ox[i] = (1 if pi == s else -1, ox[i][1])
        sig.append((s, s))
    return ox, sig


N_FFT = 64
HOP = 49
NMAT = 95
HI16 = 0xFFFF0000
YU = 6
ZA = 40


def _f32(u):
    return pltpu.bitcast(u, jnp.float32)


def _half(u, p):
    return _f32(u << 16) if p == 0 else _f32(u & jnp.uint32(HI16))


def _pack(a, b):
    return pltpu.pack_elementwise([a, b], packed_dtype=jnp.bfloat16)


@functools.lru_cache(maxsize=None)
def _codelets():
    N = N_FFT
    c = {}
    c['x32'] = _sub_rfft(32)
    c['x16'] = _sub_rfft(16)
    gx, ox = _combine(N, False, (c['x32'][2], c['x16'][2], c['x16'][2]))
    sig = None
    for p, taps in ((0, 16), (1, 15)):
        e = _sub_rfft(32, (taps + 1) // 2)
        o1 = _sub_rfft(16, (taps + 2) // 4)
        o3 = _sub_rfft(16, taps // 4)
        gw, ow = _combine(N, True, (e[2], o1[2], o3[2]))
        oxp, sig = _balance_signs(gx, ox, gw, ow, N, sig)
        c['w', p] = (e, o1, o3, gw, [(1, o[1]) for o in ow])
        c['xc', p] = (gx, oxp)
    src = [(sig[0][0], 0), (sig[0][1], 1)] + [(sig[k][0], 2 * k + t) for k in range(1, N // 2) for t in range(2)]
    gi, oU, o1, o3 = _inv_split(N, src)
    rU, sU = _unsigned(oU)
    r1, s1 = _unsigned(o1)
    r3, s3 = _unsigned(o3)
    assert (len(rU), len(r1), len(r3)) == (32, 16, 16)
    c['inv'] = (gi, rU + r1 + r3)
    c['iu'] = _sub_irfft(32, (HOP + 1) // 2, sU)
    c['i1'] = _sub_irfft(16, (HOP + 2) // 4, s1)
    c['i3'] = _sub_irfft(16, HOP // 4, s3)
    return c


def _two_half_fft(ld, st, out, subs, comb):
    (ge, oe, _), (g1, o1, _), (g3, o3, _) = subs

    def stage(base):
        def f(i, v):
            st[base + i] = v
        return f
    ge.emit(oe, lambda i: ld(0, 2 * i), store=stage(0))
    g1.emit(o1, lambda i: ld(0, 4 * i + 1), store=stage(32))
    g3.emit(o3, lambda i: ld(0, 4 * i + 3), store=stage(48))
    ge.emit(oe, lambda i: ld(1, 2 * i), store=stage(64))
    r1 = g1.emit(o1, lambda i: ld(1, 4 * i + 1))
    r3 = g3.emit(o3, lambda i: ld(1, 4 * i + 3))

    def ldc(i):
        if i < 32:
            b = st[64 + i]
        elif i < 48:
            b = r1[i - 32]
        else:
            b = r3[i - 48]
        return jnp.concatenate([st[i], b], axis=0)
    comb[0].emit(comb[1], ldc, store=lambda i, v: out(i, _pack(v[:8], v[8:])))


def _kernel(x_hbm, w_hbm, g_ref, b_ref, o_hbm,
            xbuf, wbuf, xh, wh, acc0, acc1, acc2, acc3, stx, stw, sty, stat, obuf, sem_x, sem_w, sem_o,
            *, B, T, D, K, L, RB):
    cod = _codelets()
    accs = (acc0, acc1, acc2, acc3)
    R = B * RB
    NG = R // 16
    NJ = D // 128
    XB = RB * HOP
    TH = T // 2
    NW = 8 * NJ
    GB = RB // 8
    GL = 8 * HOP

    def x_copies(j, slot):
        xv = xbuf.bitcast(jnp.bfloat16)
        return [pltpu.make_async_copy(
            x_hbm.at[b, :, pl.ds(j * 128, 128)],
            xv.at[slot, pl.ds(2 * b * XB, T), :], sem_x.at[slot, b]) for b in range(B)]

    def w_copy(j, slot):
        return pltpu.make_async_copy(
            w_hbm.at[:, pl.ds(j * 128, 128), :], wbuf.bitcast(jnp.bfloat16).at[slot], sem_w.at[slot])

    def start_in(j, slot):
        w_copy(j, slot).start()
        for c in x_copies(j, slot):
            c.start()

    def wait_in(j, slot):
        w_copy(j, slot).wait()
        for c in x_copies(j, slot):
            c.wait()

    def x_fft(G, p, xslot, so):
        def ld(e, n):
            return _half(xbuf[xslot, pl.ds(G * (16 * HOP) + HOP * e + n, 8, stride=2 * HOP), :], p)

        def out(i, v):
            xh[so, i, pl.ds(pl.multiple_of(G * 8, 8), 8), :] = v
        _two_half_fft(ld, stx, out, (cod['x32'], cod['x16'], cod['x16']), cod['xc', p])

    def w_fft(t, p, wslot, so):
        rs = pl.ds(pl.multiple_of((t // NJ) * 8, 8), 8)
        cs = pl.ds(pl.multiple_of((t % NJ) * 128, 128), 128)

        def ld(e, j):
            return _half(wbuf[wslot, 2 * j + p, rs, cs], e)

        def out(i, v):
            wh[so, i, rs, cs] = v
        e, o1, o3, gw, ow = cod['w', p]
        _two_half_fft(ld, stw, out, (e, o1, o3), (gw, ow))

    def dot(si, i, q=None):
        cs = slice(None) if q is None else pl.ds(q * 128, 128)
        a = pltpu.bitcast(xh[si, i], jnp.bfloat16)
        b = pltpu.bitcast(wh[si, i, :, cs], jnp.bfloat16)
        return jnp.dot(a, b, preferred_element_type=jnp.float32)

    def acc_add(i, v, q):
        if q is None:
            for t in range(NJ):
                accs[t][i] = accs[t][i] + v[:, t * 128:(t + 1) * 128]
        else:
            accs[q][i] = accs[q][i] + v

    def mm_bin(k, si, q=None):
        r0 = dot(si, 3 * k - 1, q)
        r1 = dot(si, 3 * k, q)
        r2 = dot(si, 3 * k + 1, q)
        acc_add(2 * k, r0 + r1, q)
        acc_add(2 * k + 1, r0 + r2, q)

    def mm_real(si, q=None):
        acc_add(0, dot(si, 0, q), q)
        acc_add(1, dot(si, 1, q), q)

    def chunk(si, nxt):
        p, islot = nxt
        mm_real(si)
        w_fft(0, p, islot, 1 - si)

        def body_a(i, c):
            mm_bin(1 + jax.lax.rem(i, 31), si)
            w_fft(1 + i, p, islot, 1 - si)
            x_fft(i, p, islot, 1 - si)
            return c
        jax.lax.fori_loop(0, NG, body_a, 0)

        def body_b(i, c):
            mm_bin(1 + jax.lax.rem(i, 31), si)
            w_fft(1 + i, p, islot, 1 - si)
            return c
        jax.lax.fori_loop(NG, NW - 1, body_b, 0)

    with jax.named_scope("ph_init"):
        start_in(0, 0)

        def zero_acc(i, c):
            for a in accs:
                a[i] = jnp.zeros(a.shape[1:], jnp.float32)
            return c
        jax.lax.fori_loop(0, ZA, zero_acc, 0)
        for slot in range(2):
            for b in range(B):
                hi = (b + 1) * XB if b + 1 < B else xbuf.shape[1]
                xbuf[slot, pl.ds(b * XB + TH, hi - b * XB - TH), :] = jnp.zeros(
                    (hi - b * XB - TH, 128), jnp.uint32)
    with jax.named_scope("ph_prow"):
        w_copy(0, 0).wait()

        def pro_w(t, c):
            w_fft(t, 0, 0, 0)
            return c
        jax.lax.fori_loop(0, NW, pro_w, 0)
        jax.lax.fori_loop(ZA, N_FFT, zero_acc, 0)
    with jax.named_scope("ph_prox"):
        def pro_x(G, c):
            x_fft(G, 0, 0, 0)
            return c
        xc = x_copies(0, 0)
        g_split = (XB - N_FFT) // (16 * HOP)
        xc[0].wait()
        jax.lax.fori_loop(0, g_split, pro_x, 0)
        xc[1].wait()
        start_in(1, 1)
        jax.lax.fori_loop(g_split, NG, pro_x, 0)

    def jstep(j, c):
        islot = j % 2
        chunk(0, (1, islot))
        wait_in(j + 1, 1 - islot)

        @pl.when(j + 2 < NJ)
        def _():
            start_in(j + 2, islot)
        chunk(1, (0, 1 - islot))
        return c
    with jax.named_scope("ph_main"):
        jax.lax.fori_loop(0, NJ - 1, jstep, 0)
        chunk(0, (1, (NJ - 1) % 2))

    gi, oi = cod['inv']
    inv_n = 1.0 / N_FFT
    c0 = 2.0 * 0.7978845608028654
    c1 = 8.0 * 0.7978845608028654 * 0.044715
    ov = obuf.bitcast(jnp.bfloat16)

    def y_fft(g8, q, u):
        rs = pl.ds(pl.multiple_of(g8 * 8, 8), 8)
        acc = accs[q]
        kept = {}

        def st1(i, v):
            if i < 32:
                sty[u, i] = v
            else:
                kept[i] = v
        gi.emit(oi, lambda i: acc[i, rs, :], store=st1)
        s = [None, None]

        def fin(n, v):
            acc[n, rs, :] = v
            s[0] = v if s[0] is None else s[0] + v
            s[1] = v * v if s[1] is None else s[1] + v * v
        cod['i1'][0].emit(cod['i1'][1], lambda i: kept[32 + i], store=lambda i, o: fin(4 * i + 1, o))
        cod['i3'][0].emit(cod['i3'][1], lambda i: kept[48 + i], store=lambda i, o: fin(4 * i + 3, o))
        cod['iu'][0].emit(cod['iu'][1], lambda i: sty[u, i], store=lambda i, o: fin(2 * i, o))
        b = g8 // GB
        stat[2 * b] = stat[2 * b] + s[0]
        stat[2 * b + 1] = stat[2 * b + 1] + s[1]

    def stats_finish(q):
        cs = pl.ds(q * 128, 128)
        for b in range(B):
            s1 = stat[2 * b]
            s2 = stat[2 * b + 1]
            for g in range(L // GL, GB):
                wrow = jax.lax.broadcasted_iota(jnp.int32, (8, 128), 0) * HOP
                for n in range(HOP):
                    v = accs[q][n, pl.ds((b * GB + g) * 8, 8), :]
                    v = jnp.where(wrow >= L - g * GL - n, v, 0.0)
                    s1 = s1 - v
                    s2 = s2 - v * v
            s1 = jnp.sum(s1, axis=0, keepdims=True) * (inv_n / L)
            s2 = jnp.sum(s2, axis=0, keepdims=True) * (inv_n * inv_n / L)
            var = jnp.maximum(s2 - s1 * s1, 0.0)
            sc = jax.lax.rsqrt(var + 1e-5) * g_ref[:, cs].astype(jnp.float32)
            sh = b_ref[:, cs].astype(jnp.float32) - s1 * sc
            stat[2 * B + 2 * b] = jnp.broadcast_to(sc * (0.5 * inv_n), (8, 128))
            stat[2 * B + 2 * b + 1] = jnp.broadcast_to(sh * 0.5, (8, 128))

    def out_copy(q, g, rows):
        return pltpu.make_async_copy(
            ov.at[q % 2, pl.ds(g * GL, rows)], o_hbm.at[pl.ds(g * GL, rows), q], sem_o.at[q % 2])

    def out_wait(q):
        pltpu.make_async_copy(ov.at[q % 2, pl.ds(0, L)], o_hbm.at[:, q], sem_o.at[q % 2]).wait()

    def out_fill(q, g):
        par = [(stat[2 * B + 2 * b], stat[2 * B + 2 * b + 1]) for b in range(B)]
        for n in range(HOP):
            r = []
            for b in range(B):
                h = accs[q][n, pl.ds(pl.multiple_of((b * GB + g) * 8, 8), 8), :]
                y = h * par[b][0] + par[b][1]
                z = ((y * y) * c1 + c0) * y
                r.append(y * jnp.tanh(z) + y)
            obuf[q % 2, pl.ds(g * GL + n, 8, stride=HOP), 0, :] = _pack(r[0], r[1])

    def out_tile(q):
        stats_finish(q)
        if q >= 2:
            out_wait(q - 2)

        def body(g, c):
            out_fill(q, g)
            out_copy(q, g, GL).start()
            return c
        jax.lax.fori_loop(0, L // GL, body, 0)
        for g in range(L // GL, pl.cdiv(L, GL)):
            out_fill(q, g)
            out_copy(q, g, L - g * GL).start()

    def zero_stat():
        for i in range(2 * B):
            stat[i] = jnp.zeros((8, 128), jnp.float32)

    def tail_phase(qm, qy):
        if qy is not None:
            zero_stat()
        if qm is not None:
            mm_real(1, qm)
            for k in range(1, 4):
                mm_bin(k, 1, qm)

        def body(i, c):
            if qm is not None:
                for k in range(4):
                    mm_bin(4 * i + k, 1, qm)
            if qy is not None:
                for u in range(YU):
                    y_fft(YU * (i - 1) + u, qy, u)
            return c
        jax.lax.fori_loop(1, N_FFT // 8, body, 0)

    with jax.named_scope("ph_tail"):
        for q in range(NJ + 1):
            tail_phase(q if q < NJ else None, q - 1 if q >= 1 else None)
            if q >= 1:
                out_tile(q - 1)
        for q in range(max(NJ - 2, 0), NJ):
            out_wait(q)


@jax.jit
def pallas_standalone__self_sup_conv_stem_wavlm__speech_kernel(x, w, gn_gamma, gn_beta):
    B, T, D = x.shape
    K = w.shape[0]
    s = 2
    L = (T - K) // s + 1
    assert B == 2 and K == 31 and D == 512 and T % 16 == 0
    nwin = pl.cdiv(L, HOP)
    RB = pl.cdiv(nwin, 8) * 8
    R = B * RB
    NJ = D // 128
    xrows = pl.cdiv(R * HOP + N_FFT, 8) * 8
    kern = functools.partial(_kernel, B=B, T=T, D=D, K=K, L=L, RB=RB)
    out = pl.pallas_call(
        kern,
        in_specs=[
            pl.BlockSpec(memory_space=pl.ANY),
            pl.BlockSpec(memory_space=pl.ANY),
            pl.BlockSpec(memory_space=pltpu.VMEM),
            pl.BlockSpec(memory_space=pltpu.VMEM),
        ],
        out_specs=pl.BlockSpec(memory_space=pl.ANY),
        out_shape=jax.ShapeDtypeStruct((L, NJ, B, 128), x.dtype),
        scratch_shapes=[
            pltpu.VMEM((2, xrows, 128), jnp.uint32),
            pltpu.VMEM((2, K, 64, D), jnp.uint32),
            pltpu.VMEM((2, NMAT, R // 2, 128), jnp.uint32),
            pltpu.VMEM((2, NMAT, 64, D), jnp.uint32),
            pltpu.VMEM((N_FFT, R, 128), jnp.float32),
            pltpu.VMEM((N_FFT, R, 128), jnp.float32),
            pltpu.VMEM((N_FFT, R, 128), jnp.float32),
            pltpu.VMEM((N_FFT, R, 128), jnp.float32),
            pltpu.VMEM((96, 8, 128), jnp.float32),
            pltpu.VMEM((96, 8, 128), jnp.float32),
            pltpu.VMEM((YU, 32, 8, 128), jnp.float32),
            pltpu.VMEM((4 * B, 8, 128), jnp.float32),
            pltpu.VMEM((2, RB * HOP, 1, 128), jnp.uint32),
            pltpu.SemaphoreType.DMA((2, B)),
            pltpu.SemaphoreType.DMA((2,)),
            pltpu.SemaphoreType.DMA((2,)),
        ],
        compiler_params=pltpu.CompilerParams(vmem_limit_bytes=124 * 1024 * 1024),
    )(x, w, gn_gamma.reshape(1, D), gn_beta.reshape(1, D))
    return jnp.transpose(out, (2, 0, 1, 3)).reshape(B, L, D)
```

```python
import functools
import math

import jax
import jax.numpy as jnp
import jax.experimental.pallas as pl
import jax.experimental.pallas.tpu as pltpu


class _Dag:
    def __init__(self):
        self.nodes = []
        self.memo = {}

    def _node(self, key):
        if key not in self.memo:
            self.memo[key] = len(self.nodes)
            self.nodes.append(key)
        return self.memo[key]

    def inp(self, i, sign=1):
        return (sign, self._node(('in', i)))

    @staticmethod
    def neg(a):
        return None if a is None else (-a[0], a[1])

    def add(self, a, b):
        if a is None:
            return b
        if b is None:
            return a
        (sa, na), (sb, nb) = a, b
        if sa == sb:
            return (sa, self._node(('add', min(na, nb), max(na, nb))))
        if sa > 0:
            return (1, self._node(('sub', na, nb)))
        return (1, self._node(('sub', nb, na)))

    def sub(self, a, b):
        return self.add(a, self.neg(b))

    def mul(self, a, c):
        if a is None or c == 0.0:
            return None
        s, n = a
        c = c * s
        if c == 1.0:
            return (1, n)
        if c == -1.0:
            return (-1, n)
        return (1 if c > 0 else -1, self._node(('mul', n, abs(c))))

    def cadd(self, a, b):
        return (self.add(a[0], b[0]), self.add(a[1], b[1]))

    def csub(self, a, b):
        return (self.sub(a[0], b[0]), self.sub(a[1], b[1]))

    def conj(self, a):
        return (a[0], self.neg(a[1]))

    def cmul_const(self, a, c, s):
        re, im = a
        if re is None or im is None or c == 0.0 or s == 0.0 or abs(c) != abs(s):
            return (self.sub(self.mul(re, c), self.mul(im, s)),
                    self.add(self.mul(re, s), self.mul(im, c)))
        t1 = self.sub(self.mul(re, math.copysign(1, c)), self.mul(im, math.copysign(1, s)))
        t2 = self.add(self.mul(re, math.copysign(1, s)), self.mul(im, math.copysign(1, c)))
        return (self.mul(t1, abs(c)), self.mul(t2, abs(c)))

    @staticmethod
    def tw(k, n):
        k %= n
        if (8 * k) % n == 0:
            r = math.sqrt(0.5)
            return [(1.0, 0.0), (r, -r), (0.0, -1.0), (-r, -r),
                    (-1.0, 0.0), (-r, r), (0.0, 1.0), (r, r)][8 * k // n]
        return (math.cos(2 * math.pi * k / n), -math.sin(2 * math.pi * k / n))

    def rfft_combine(self, e, o1, o3, n, emit_bin=None):
        q = n // 4
        out = [None] * (n // 2 + 1)

        def E(k):
            return e[k] if k <= q else self.conj(e[n // 2 - k])

        def done(*ks):
            if emit_bin is not None:
                for kk in ks:
                    emit_bin(kk, out)
        s0 = self.add(o1[0][0], o3[0][0])
        d0 = self.sub(o1[0][0], o3[0][0])
        out[0] = (self.add(e[0][0], s0), None)
        out[n // 2] = (self.sub(e[0][0], s0), None)
        out[q] = (e[q][0], self.neg(d0))
        done(0, n // 2, q)
        for k in range(1, q // 2 + 1):
            if 2 * k == q:
                a1, a3 = o1[k][0], o3[k][0]
                r = math.sqrt(0.5)
                S = (self.mul(self.sub(a1, a3), r), self.neg(self.mul(self.add(a1, a3), r)))
                out[k] = self.cadd(E(k), S)
                out[n // 2 - k] = self.conj(self.csub(E(k), S))
                done(k, n // 2 - k)
                continue
            z1 = self.cmul_const(o1[k], *self.tw(k, n))
            z3 = self.cmul_const(o3[k], *self.tw(3 * k, n))
            S = self.cadd(z1, z3)
            Dd = self.csub(z1, z3)
            mi_d = (Dd[1], self.neg(Dd[0]))
            out[k] = self.cadd(E(k), S)
            out[n // 2 - k] = self.conj(self.csub(E(k), S))
            out[q + k] = self.cadd(E(q + k), mi_d)
            out[q - k] = self.conj(self.csub(E(q + k), mi_d))
            done(k, n // 2 - k, q + k, q - k)
        return out

    def rfft(self, x):
        n = len(x)
        if n == 1:
            return [(x[0], None)]
        if n == 2:
            return [(self.add(x[0], x[1]), None), (self.sub(x[0], x[1]), None)]
        e = self.rfft(x[0::2])
        o1 = self.rfft(x[1::4])
        o3 = self.rfft(x[3::4])
        return self.rfft_combine(e, o1, o3, n)

    def irfft_split(self, X):
        n = 2 * (len(X) - 1)
        q, h = n // 4, n // 2
        U = [None] * (q + 1)
        z1 = [None] * (n // 8 + 1)
        z3 = [None] * (n // 8 + 1)
        U[0] = (self.add(X[0][0], X[h][0]), None)
        U[q] = (self.mul(X[q][0], 2.0), None)
        a0 = self.sub(X[0][0], X[h][0])
        ib0 = self.neg(self.mul(X[q][1], 2.0))
        z1[0] = (self.add(a0, ib0), None)
        z3[0] = (self.sub(a0, ib0), None)
        for k in range(1, n // 8 + 1):
            U[k] = self.cadd(X[k], self.conj(X[h - k]))
            A = self.csub(X[k], self.conj(X[h - k]))
            if 8 * k == n:
                r2 = math.sqrt(2.0)
                z1[k] = (self.mul(self.sub(A[0], A[1]), r2), None)
                z3[k] = (self.mul(self.add(A[0], A[1]), -r2), None)
                continue
            U[q - k] = self.cadd(X[q - k], self.conj(X[q + k]))
            Bk = self.csub(X[q + k], self.conj(X[q - k]))
            iB = (self.neg(Bk[1]), Bk[0])
            z1[k] = self.cmul_const(self.cadd(A, iB), *self.tw(-k, n))
            z3[k] = self.cmul_const(self.csub(A, iB), *self.tw(-3 * k, n))
        return U, z1, z3

    def irfft(self, X):
        if len(X) == 1:
            return [X[0][0]]
        if len(X) == 2:
            return [self.add(X[0][0], X[1][0]), self.sub(X[0][0], X[1][0])]
        n = 2 * (len(X) - 1)
        if n == 4:
            U = [(self.add(X[0][0], X[2][0]), None), (self.mul(X[1][0], 2.0), None)]
            a0 = self.sub(X[0][0], X[2][0])
            ib0 = self.neg(self.mul(X[1][1], 2.0))
            z1 = [(self.add(a0, ib0), None)]
            z3 = [(self.sub(a0, ib0), None)]
        else:
            U, z1, z3 = self.irfft_split(X)
        out = [None] * n
        out[0::2] = self.irfft(U)
        out[1::4] = self.irfft(z1)
        out[3::4] = self.irfft(z3)
        return out

    def emit(self, outs, load, store=None, zero=None):
        nodes = self.nodes
        uses = {}
        need = set()
        stack = [o[1] for o in outs if o is not None]
        while stack:
            t = stack.pop()
            if t in need:
                continue
            need.add(t)
            key = nodes[t]
            if key[0] != 'in':
                for d in (key[1:3] if key[0] != 'mul' else key[1:2]):
                    uses[d] = uses.get(d, 0) + 1
                    stack.append(d)
        by_node = {}
        for i, o in enumerate(outs):
            if o is not None:
                by_node.setdefault(o[1], []).append((i, o[0]))
        val = {}
        res = [None] * len(outs)

        def get(t):
            if t not in val:
                val[t] = load(nodes[t][1])
            return val[t]

        def put(i, v):
            if store is not None:
                store(i, v)
            else:
                res[i] = v

        def fin(t, flipped):
            for i, sg in by_node.get(t, ()):
                put(i, val[t] if (sg > 0) != flipped else -val[t])
        for t, key in enumerate(nodes):
            if t not in need or key[0] == 'in':
                continue
            flipped = False
            if key[0] == 'add':
                val[t] = get(key[1]) + get(key[2])
            elif key[0] == 'sub':
                if uses.get(t, 0) == 0 and all(sg < 0 for _, sg in by_node[t]):
                    flipped = True
                    first, second = get(key[1]), get(key[2])
                    val[t] = second - first
                else:
                    val[t] = get(key[1]) - get(key[2])
            else:
                if uses.get(t, 0) == 0 and all(sg < 0 for _, sg in by_node[t]):
                    flipped = True
                    val[t] = get(key[1]) * (-key[2])
                else:
                    val[t] = get(key[1]) * key[2]
            fin(t, flipped)
        for i, o in enumerate(outs):
            if o is None:
                put(i, zero())
            elif nodes[o[1]][0] == 'in':
                v = get(o[1])
                put(i, v if o[0] > 0 else -v)
        return res


def _spec_flat(X):
    n2 = len(X) - 1
    return [X[0][0], X[n2][0]] + [v for k in range(1, n2) for v in X[k]]


def _spec_in(g, base, n, src=None):
    def one(i):
        if src is None:
            return g.inp(base + i)
        if src[i] is None:
            return None
        return g.inp(base + src[i][1], src[i][0])
    return ([(one(0), None)] + [(one(2 * k), one(2 * k + 1)) for k in range(1, n // 2)] + [(one(1), None)])


def _unsigned(outs):
    slot, raw, src = {}, [], []
    for o in outs:
        if o is None:
            src.append(None)
            continue
        if o[1] not in slot:
            slot[o[1]] = len(raw)
            raw.append((1, o[1]))
        src.append((o[0], slot[o[1]]))
    return raw, src


def _sub_rfft(n, taps=None):
    g = _Dag()
    X = g.rfft([g.inp(i) if taps is None or i < taps else None for i in range(n)])
    raw, src = _unsigned(_spec_flat(X))
    return g, raw, src


def _combine(N, weights, srcs, flips=None):
    g = _Dag()
    e = _spec_in(g, 0, N // 2, srcs[0])
    o1 = _spec_in(g, N // 2, N // 4, srcs[1])
    o3 = _spec_in(g, 3 * N // 4, N // 4, srcs[2])
    outs = [None] * (3 * (N // 2) - 1)

    def emit_bin(k, out):
        a, b = out[k]
        if k == 0:
            outs[0] = a
        elif k == N // 2:
            outs[1] = a
        elif weights:
            outs[3 * k - 1:3 * k + 2] = [g.sub(a, b), b, a]
        else:
            outs[3 * k - 1:3 * k + 2] = [a, g.add(a, b), g.sub(b, a)]
    g.rfft_combine(e, o1, o3, N, emit_bin)
    return g, outs


def _inv_split(N, src):
    g = _Dag()
    U, z1, z3 = g.irfft_split(_spec_in(g, 0, N, src))
    return g, _spec_flat(U), _spec_flat(z1), _spec_flat(z3)


def _sub_irfft(n, keep, src):
    g = _Dag()
    y = g.irfft(_spec_in(g, 0, n, src))
    return g, y[:keep]


def _flippable(g, outs):
    used = set()
    for key in g.nodes:
        if key[0] != 'in':
            used.update(key[1:3] if key[0] != 'mul' else key[1:2])
    cnt = {}
    for o in outs:
        cnt[o[1]] = cnt.get(o[1], 0) + 1
    return [g.nodes[o[1]][0] in ('sub', 'mul') and o[1] not in used and cnt[o[1]] == 1 for o in outs]


def _balance_signs(gx, ox, gw, ow, N, force=None):
    fx = _flippable(gx, ox)
    ox = list(ox)
    sig = []
    for k in range(N // 2):
        idx = [0] if k == 0 else [3 * k - 1, 3 * k, 3 * k + 1]
        if k == 0:
            s01 = (ox[0][0] * ow[0][0], ox[1][0] * ow[1][0]) if force is None else force[0]
            ox[0] = (ox[0][0] * ow[0][0] * s01[0], ox[0][1])
            ox[1] = (ox[1][0] * ow[1][0] * s01[1], ox[1][1])
            sig.append(s01)
            continue
        p = [ox[i][0] * ow[i][0] for i in idx]
        best = None
        for s in (1, -1):
            cost = sum(0 if (pi == s or fx[i]) else 1 for pi, i in zip(p, idx))
            if best is None or cost < best[0]:
                best = (cost, s)
        s = best[1] if force is None else force[k][0]
        for pi, i in zip(p, idx):
            ox[i] = (1 if pi == s else -1, ox[i][1])
        sig.append((s, s))
    return ox, sig


N_FFT = 64
HOP = 49
NMAT = 95
HI16 = 0xFFFF0000
OU = 3
YU = 6
ZA = 40


def _f32(u):
    return pltpu.bitcast(u, jnp.float32)


def _half(u, p):
    return _f32(u << 16) if p == 0 else _f32(u & jnp.uint32(HI16))


def _pack(a, b):
    return pltpu.pack_elementwise([a, b], packed_dtype=jnp.bfloat16)


@functools.lru_cache(maxsize=None)
def _codelets():
    N = N_FFT
    c = {}
    c['x32'] = _sub_rfft(32)
    c['x16'] = _sub_rfft(16)
    gx, ox = _combine(N, False, (c['x32'][2], c['x16'][2], c['x16'][2]))
    sig = None
    for p, taps in ((0, 16), (1, 15)):
        e = _sub_rfft(32, (taps + 1) // 2)
        o1 = _sub_rfft(16, (taps + 2) // 4)
        o3 = _sub_rfft(16, taps // 4)
        gw, ow = _combine(N, True, (e[2], o1[2], o3[2]))
        oxp, sig = _balance_signs(gx, ox, gw, ow, N, sig)
        c['w', p] = (e, o1, o3, gw, [(1, o[1]) for o in ow])
        c['xc', p] = (gx, oxp)
    src = [(sig[0][0], 0), (sig[0][1], 1)] + [(sig[k][0], 2 * k + t) for k in range(1, N // 2) for t in range(2)]
    gi, oU, o1, o3 = _inv_split(N, src)
    rU, sU = _unsigned(oU)
    r1, s1 = _unsigned(o1)
    r3, s3 = _unsigned(o3)
    assert (len(rU), len(r1), len(r3)) == (32, 16, 16)
    c['inv'] = (gi, rU + r1 + r3)
    c['iu'] = _sub_irfft(32, (HOP + 1) // 2, sU)
    c['i1'] = _sub_irfft(16, (HOP + 2) // 4, s1)
    c['i3'] = _sub_irfft(16, HOP // 4, s3)
    return c


def _two_half_fft(ld, st, out, subs, comb):
    (ge, oe, _), (g1, o1, _), (g3, o3, _) = subs
    kept = {}

    def stage(base):
        def f(i, v):
            st[base + i] = v
        return f

    def p0():
        ge.emit(oe, lambda i: ld(0, 2 * i), store=stage(0))

    def p1():
        g1.emit(o1, lambda i: ld(0, 4 * i + 1), store=stage(32))
        g3.emit(o3, lambda i: ld(0, 4 * i + 3), store=stage(48))

    def p2():
        ge.emit(oe, lambda i: ld(1, 2 * i), store=stage(64))

    def p3():
        kept[1] = g1.emit(o1, lambda i: ld(1, 4 * i + 1))
        kept[3] = g3.emit(o3, lambda i: ld(1, 4 * i + 3))

    def ldc(i):
        if i < 32:
            b = st[64 + i]
        elif i < 48:
            b = kept[1][i - 32]
        else:
            b = kept[3][i - 48]
        return jnp.concatenate([st[i], b], axis=0)

    def p4(defer=None):
        if defer is None:
            comb[0].emit(comb[1], ldc, store=lambda i, v: out(i, _pack(v[:8], v[8:])))
        else:
            comb[0].emit(comb[1], ldc, store=lambda i, v: defer.append(
                functools.partial(out, i, _pack(v[:8], v[8:]))))
    return [p0, p1, p2, p3, p4]


def _kernel(x_hbm, w_hbm, g_ref, b_ref, o_hbm,
            xbuf, wbuf, xh, wh, acc0, acc1, acc2, acc3, stx, stw, stx2, stw2, sty, stat, obuf, sem_x, sem_w, sem_o,
            *, B, T, D, K, L, RB):
    cod = _codelets()
    accs = (acc0, acc1, acc2, acc3)
    R = B * RB
    NG = R // 16
    NJ = D // 128
    XB = RB * HOP
    TH = T // 2
    NW = 8 * NJ
    GB = RB // 8
    GL = 8 * HOP

    def x_copies(j, slot):
        xv = xbuf.bitcast(jnp.bfloat16)
        return [pltpu.make_async_copy(
            x_hbm.at[b, :, pl.ds(j * 128, 128)],
            xv.at[slot, pl.ds(2 * b * XB, T), :], sem_x.at[slot, b]) for b in range(B)]

    def w_copy(j, slot):
        return pltpu.make_async_copy(
            w_hbm.at[:, pl.ds(j * 128, 128), :], wbuf.bitcast(jnp.bfloat16).at[slot], sem_w.at[slot])

    def start_in(j, slot):
        w_copy(j, slot).start()
        for c in x_copies(j, slot):
            c.start()

    def wait_in(j, slot):
        w_copy(j, slot).wait()
        for c in x_copies(j, slot):
            c.wait()

    def x_fft(G, p, xslot, so, stx=stx):
        def ld(e, n):
            return _half(xbuf[xslot, pl.ds(G * (16 * HOP) + HOP * e + n, 8, stride=2 * HOP), :], p)

        def out(i, v):
            xh[so, i, pl.ds(pl.multiple_of(G * 8, 8), 8), :] = v
        return _two_half_fft(ld, stx, out, (cod['x32'], cod['x16'], cod['x16']), cod['xc', p])

    def w_fft(t, p, wslot, so, stw=stw):
        rs = pl.ds(pl.multiple_of((t // NJ) * 8, 8), 8)
        cs = pl.ds(pl.multiple_of((t % NJ) * 128, 128), 128)

        def ld(e, j):
            return _half(wbuf[wslot, 2 * j + p, rs, cs], e)

        def out(i, v):
            wh[so, i, rs, cs] = v
        e, o1, o3, gw, ow = cod['w', p]
        return _two_half_fft(ld, stw, out, (e, o1, o3), (gw, ow))

    def run(parts):
        for f in parts:
            f()

    def dot(si, i, q=None):
        cs = slice(None) if q is None else pl.ds(q * 128, 128)
        a = pltpu.bitcast(xh[si, i], jnp.bfloat16)
        b = pltpu.bitcast(wh[si, i, :, cs], jnp.bfloat16)
        return jnp.dot(a, b, preferred_element_type=jnp.float32)

    def acc_add(i, v, q):
        if q is None:
            for t in range(NJ):
                accs[t][i] = accs[t][i] + v[:, t * 128:(t + 1) * 128]
        else:
            accs[q][i] = accs[q][i] + v

    def mm_bin(k, si, q=None):
        r0 = dot(si, 3 * k - 1, q)
        r1 = dot(si, 3 * k, q)
        r2 = dot(si, 3 * k + 1, q)
        acc_add(2 * k, r0 + r1, q)
        acc_add(2 * k + 1, r0 + r2, q)

    def mm_real(si, q=None):
        acc_add(0, dot(si, 0, q), q)
        acc_add(1, dot(si, 1, q), q)

    def chunk(si, nxt):
        p, islot = nxt
        mm_real(si)
        run(w_fft(0, p, islot, 1 - si))

        def body(prog, base, un):
            def f(i, c):
                i0 = base + i * un
                k = 1 + jax.lax.rem(i0, 31)
                k2 = 1 + jax.lax.rem(i0 + 1, 31)
                r = {}
                for ch in prog:
                    if ch in 'abcdef':
                        kk = k if ch in 'abc' else k2
                        o = 'abcdef'.index(ch)
                        if o % 3 == 0:
                            r[o // 3] = dot(si, 3 * kk - 1)
                        else:
                            acc_add(2 * kk + o % 3 - 1, r[o // 3] + dot(si, 3 * kk + o % 3 - 1), None)
                    elif ch == 'x':
                        run(x_fft(i0, p, islot, 1 - si))
                    elif ch == 'y':
                        run(x_fft(i0 + 1, p, islot, 1 - si, stx2))
                    elif ch == 'w':
                        run(w_fft(1 + i0, p, islot, 1 - si))
                    elif ch == 'v':
                        run(w_fft(2 + i0, p, islot, 1 - si, stw2))
                return c
            return f
        pb = 'adbwcevf'
        jax.lax.fori_loop(0, NG, body('abxcw', 0, 1), 0)
        un = 2 if 'd' in pb else 1
        jax.lax.fori_loop(0, (NW - 1 - NG) // un, body(pb, NG, un), 0)

    with jax.named_scope("ph_init"):
        start_in(0, 0)

        def zero_acc(i, c):
            for a in accs:
                a[i] = jnp.zeros(a.shape[1:], jnp.float32)
            return c
        jax.lax.fori_loop(0, ZA, zero_acc, 0)
        for slot in range(2):
            for b in range(B):
                hi = (b + 1) * XB if b + 1 < B else xbuf.shape[1]
                xbuf[slot, pl.ds(b * XB + TH, hi - b * XB - TH), :] = jnp.zeros(
                    (hi - b * XB - TH, 128), jnp.uint32)
    with jax.named_scope("ph_prow"):
        w_copy(0, 0).wait()

        def pro_w(t, c):
            run(w_fft(t, 0, 0, 0))
            return c
        jax.lax.fori_loop(0, NW, pro_w, 0)
        jax.lax.fori_loop(ZA, N_FFT, zero_acc, 0)
    with jax.named_scope("ph_prox"):
        def pro_x(G, c):
            run(x_fft(G, 0, 0, 0))
            return c
        xc = x_copies(0, 0)
        g_split = (XB - N_FFT) // (16 * HOP)
        xc[0].wait()
        jax.lax.fori_loop(0, g_split, pro_x, 0)
        xc[1].wait()
        start_in(1, 1)
        jax.lax.fori_loop(g_split, NG, pro_x, 0)

    def jstep(j, c):
        islot = j % 2
        chunk(0, (1, islot))
        wait_in(j + 1, 1 - islot)

        @pl.when(j + 2 < NJ)
        def _():
            start_in(j + 2, islot)
        chunk(1, (0, 1 - islot))
        return c
    with jax.named_scope("ph_main"):
        jax.lax.fori_loop(0, NJ - 1, jstep, 0)
        chunk(0, (1, (NJ - 1) % 2))

    gi, oi = cod['inv']
    inv_n = 1.0 / N_FFT
    c0 = 2.0 * 0.7978845608028654
    c1 = 8.0 * 0.7978845608028654 * 0.044715
    ov = obuf.bitcast(jnp.bfloat16)

    def y_fft(g8, q, u, tick=lambda: None):
        rs = pl.ds(pl.multiple_of(g8 * 8, 8), 8)
        acc = accs[q]
        kept = {}

        def st1(i, v):
            if i < 32:
                sty[u, i] = v
            else:
                kept[i] = v
            tick()
        gi.emit(oi, lambda i: acc[i, rs, :], store=st1)
        s = [None, None]

        def fin(n, v):
            acc[n, rs, :] = v
            s[0] = v if s[0] is None else s[0] + v
            s[1] = v * v if s[1] is None else s[1] + v * v
            tick()
        cod['i1'][0].emit(cod['i1'][1], lambda i: kept[32 + i], store=lambda i, o: fin(4 * i + 1, o))
        cod['i3'][0].emit(cod['i3'][1], lambda i: kept[48 + i], store=lambda i, o: fin(4 * i + 3, o))
        cod['iu'][0].emit(cod['iu'][1], lambda i: sty[u, i], store=lambda i, o: fin(2 * i, o))
        b = g8 // GB
        stat[2 * b] = stat[2 * b] + s[0]
        stat[2 * b + 1] = stat[2 * b + 1] + s[1]

    def stats_finish(q):
        cs = pl.ds(q * 128, 128)
        for b in range(B):
            s1 = stat[2 * b]
            s2 = stat[2 * b + 1]
            for g in range(L // GL, GB):
                wrow = jax.lax.broadcasted_iota(jnp.int32, (8, 128), 0) * HOP
                for n in range(HOP):
                    v = accs[q][n, pl.ds((b * GB + g) * 8, 8), :]
                    v = jnp.where(wrow >= L - g * GL - n, v, 0.0)
                    s1 = s1 - v
                    s2 = s2 - v * v
            s1 = jnp.sum(s1, axis=0, keepdims=True) * (inv_n / L)
            s2 = jnp.sum(s2, axis=0, keepdims=True) * (inv_n * inv_n / L)
            var = jnp.maximum(s2 - s1 * s1, 0.0)
            sc = jax.lax.rsqrt(var + 1e-5) * g_ref[:, cs].astype(jnp.float32)
            sh = b_ref[:, cs].astype(jnp.float32) - s1 * sc
            stat[2 * B + 2 * b] = jnp.broadcast_to(sc * (0.5 * inv_n), (8, 128))
            stat[2 * B + 2 * b + 1] = jnp.broadcast_to(sh * 0.5, (8, 128))

    def out_copy(q, g, rows):
        return pltpu.make_async_copy(
            ov.at[q % 2, pl.ds(g * GL, rows)], o_hbm.at[pl.ds(g * GL, rows), q], sem_o.at[q % 2])

    def out_wait(q):
        pltpu.make_async_copy(ov.at[q % 2, pl.ds(0, L)], o_hbm.at[:, q], sem_o.at[q % 2]).wait()

    def out_steps(q, g):
        par = [(stat[2 * B + 2 * b], stat[2 * B + 2 * b + 1]) for b in range(B)]

        def step(n):
            r = []
            for b in range(B):
                h = accs[q][n, pl.ds(pl.multiple_of((b * GB + g) * 8, 8), 8), :]
                y = h * par[b][0] + par[b][1]
                z = ((y * y) * c1 + c0) * y
                r.append(y * jnp.tanh(z) + y)
            obuf[q % 2, pl.ds(g * GL + n, 8, stride=HOP), 0, :] = _pack(r[0], r[1])
        return [functools.partial(step, n) for n in range(HOP)]

    def zero_stat():
        for i in range(2 * B):
            stat[i] = jnp.zeros((8, 128), jnp.float32)

    def tail_phase(qm, qy, qo):
        if qy is not None:
            zero_stat()
        if qo is not None and qo >= 2:
            out_wait(qo - 2)
        if qm is not None:
            mm_real(1, qm)
            for k in range(1, 4):
                mm_bin(k, 1, qm)

        def body(i, c):
            pend = []
            if qo is not None:
                for io in range(OU):
                    pend += out_steps(qo, OU * (i - 1) + io)
            pend.reverse()
            nt = 113 * YU
            state = [0, 0]

            mms = [functools.partial(mm_bin, 4 * i + im, 1, qm) for im in range(4)] if qm is not None else []
            mpos = [int(float(v) * nt) for v in '0.1,0.3,0.5,0.7'.split(',')]

            def tick():
                while mms and state[0] >= mpos[4 - len(mms)]:
                    mms.pop(0)()
                state[0] += 1
                while state[1] * nt < state[0] * OU * HOP and pend:
                    pend.pop()()
                    state[1] += 1
            if qy is not None:
                for iy in range(YU):
                    y_fft(YU * (i - 1) + iy, qy, iy, tick)
            while mms:
                mms.pop(0)()
            while pend:
                pend.pop()()
            if qo is not None:
                for io in range(OU - 1):
                    out_copy(qo, OU * (i - 1) + io, GL).start()
                g = OU * (i - 1) + OU - 1

                @pl.when(g < L // GL)
                def _():
                    out_copy(qo, g, GL).start()

                @pl.when(g >= L // GL)
                def _():
                    out_copy(qo, L // GL, L - (L // GL) * GL).start()
            return c
        jax.lax.fori_loop(1, N_FFT // 8, body, 0)
        if qy is not None:
            stats_finish(qy)

    with jax.named_scope("ph_tail"):
        for q in range(NJ + 2):
            tail_phase(q if q < NJ else None, q - 1 if 1 <= q <= NJ else None, q - 2 if q >= 2 else None)
        for q in range(max(NJ - 2, 0), NJ):
            out_wait(q)


@jax.jit
def pallas_standalone__self_sup_conv_stem_wavlm__speech_kernel(x, w, gn_gamma, gn_beta):
    B, T, D = x.shape
    K = w.shape[0]
    s = 2
    L = (T - K) // s + 1
    assert B == 2 and K == 31 and D == 512 and T % 16 == 0
    nwin = pl.cdiv(L, HOP)
    RB = pl.cdiv(nwin, 8) * 8
    R = B * RB
    NJ = D // 128
    xrows = pl.cdiv(R * HOP + N_FFT, 8) * 8
    kern = functools.partial(_kernel, B=B, T=T, D=D, K=K, L=L, RB=RB)
    out = pl.pallas_call(
        kern,
        in_specs=[
            pl.BlockSpec(memory_space=pl.ANY),
            pl.BlockSpec(memory_space=pl.ANY),
            pl.BlockSpec(memory_space=pltpu.VMEM),
            pl.BlockSpec(memory_space=pltpu.VMEM),
        ],
        out_specs=pl.BlockSpec(memory_space=pl.ANY),
        out_shape=jax.ShapeDtypeStruct((L, NJ, B, 128), x.dtype),
        scratch_shapes=[
            pltpu.VMEM((2, xrows, 128), jnp.uint32),
            pltpu.VMEM((2, K, 64, D), jnp.uint32),
            pltpu.VMEM((2, NMAT, R // 2, 128), jnp.uint32),
            pltpu.VMEM((2, NMAT, 64, D), jnp.uint32),
            pltpu.VMEM((N_FFT, R, 128), jnp.float32),
            pltpu.VMEM((N_FFT, R, 128), jnp.float32),
            pltpu.VMEM((N_FFT, R, 128), jnp.float32),
            pltpu.VMEM((N_FFT, R, 128), jnp.float32),
            pltpu.VMEM((96, 8, 128), jnp.float32),
            pltpu.VMEM((96, 8, 128), jnp.float32),
            pltpu.VMEM((96, 8, 128), jnp.float32),
            pltpu.VMEM((96, 8, 128), jnp.float32),
            pltpu.VMEM((YU, 32, 8, 128), jnp.float32),
            pltpu.VMEM((4 * B, 8, 128), jnp.float32),
            pltpu.VMEM((2, RB * HOP, 1, 128), jnp.uint32),
            pltpu.SemaphoreType.DMA((2, B)),
            pltpu.SemaphoreType.DMA((2,)),
            pltpu.SemaphoreType.DMA((2,)),
        ],
        compiler_params=pltpu.CompilerParams(vmem_limit_bytes=124 * 1024 * 1024),
    )(x, w, gn_gamma.reshape(1, D), gn_beta.reshape(1, D))
    return jnp.transpose(out, (2, 0, 1, 3)).reshape(B, L, D)
```
